```python
import os as _os
_os.environ.setdefault("JAX_PLATFORMS", "cpu")
import jax
import jax.numpy as jnp

def _softmax(x, axis=-1):
    return jax.nn.softmax(x, axis=axis)
def _gelu(x):
    return jax.nn.gelu(x, approximate=True)
def _silu(x):
    return jax.nn.silu(x)
def _sigmoid(x):
    return jax.nn.sigmoid(x)
def _layernorm(x, axis=-1, eps=1e-5):
    m = jnp.mean(x, axis=axis, keepdims=True)
    v = jnp.var(x, axis=axis, keepdims=True)
    return (x - m) / jnp.sqrt(v + eps)
def _scatter_add(tgt, idx, src, axis=0):
    return tgt.at[idx].add(src)
def _segment_sum(src, seg, n):
    return jax.ops.segment_sum(src, seg, n)
class _Rng:
    def __init__(self, key):
        self._k = key
    def _next(self):
        self._k, sub = jax.random.split(self._k)
        return sub
    def normal(self, shape):
        return jax.random.normal(self._next(), shape, dtype=jnp.bfloat16)
    def randint(self, lo, hi, shape):
        return jax.random.randint(self._next(), shape, lo, hi, dtype=jnp.int32)
    def uniform(self, shape, lo=0.0, hi=1.0):
        return jax.random.uniform(self._next(), shape, jnp.bfloat16, lo, hi)
    def permutation(self, n):
        return jax.random.permutation(self._next(), n)


kernel_name = 'standalone__mha_softmax__sampling'

def setup_inputs():
    _rng = _Rng(jax.random.key(int.from_bytes(__import__("os").urandom(4), "little")))
    _w = (lambda a: (lambda t: t.astype(jnp.bfloat16) if jnp.issubdtype(t.dtype, jnp.floating) else t)(jnp.asarray(a)))
    B, H, Sq, Sk, D = 8, 32, 32, 2048, 128
    return {
        "q": _w((lambda *s: _rng.normal(s) * 0.4)(B, H, Sq, D)),
        "k": _w((lambda *s: _rng.normal(s) * 0.4)(B, H, Sk, D)),
        "v": _w((lambda *s: _rng.normal(s) * 0.05)(B, H, Sk, D)),
    }

def reference(q, k, v):
    scale = q.shape[-1] ** -0.5
    scores = jnp.einsum("bhqd,bhkd->bhqk", q, k) * scale
    p = _softmax(scores, axis=-1)
    return jnp.einsum("bhqk,bhkd->bhqd", p, v)
```

```python
import math

import jax
import jax.numpy as jnp
from jax import lax
import jax.experimental.pallas as pl
import jax.experimental.pallas.tpu as pltpu

_G = 4


def _kernel(q_ref, k_ref, v_ref, o_ref):
    d = q_ref.shape[-1]
    c = (d ** -0.5) * math.log2(math.e)
    for g in range(_G):
        s = lax.dot_general(
            q_ref[g], k_ref[g], (((1,), (1,)), ((), ())),
            preferred_element_type=jnp.float32)
        m = jnp.max(s, axis=-1, keepdims=True)
        p = jnp.exp2((s - m) * c)
        l = jnp.sum(p, axis=-1, keepdims=True)
        o = jnp.dot(p.astype(jnp.bfloat16), v_ref[g],
                    preferred_element_type=jnp.float32)
        o_ref[g] = (o / l).astype(o_ref.dtype)


@jax.jit
def pallas_standalone__mha_softmax__sampling_kernel(
    q: jax.Array,
    k: jax.Array,
    v: jax.Array,
):
    B, H, Sq, D = q.shape
    Sk = k.shape[2]
    BH = B * H
    out = pl.pallas_call(
        _kernel,
        grid=(BH // _G,),
        in_specs=[
            pl.BlockSpec((_G, Sq, D), lambda i: (i, 0, 0)),
            pl.BlockSpec((_G, Sk, D), lambda i: (i, 0, 0)),
            pl.BlockSpec((_G, Sk, D), lambda i: (i, 0, 0)),
        ],
        out_specs=pl.BlockSpec((_G, Sq, D), lambda i: (i, 0, 0)),
        out_shape=jax.ShapeDtypeStruct((BH, Sq, D), q.dtype),
        compiler_params=pltpu.CompilerParams(
            dimension_semantics=("arbitrary",),
            vmem_limit_bytes=64 * 1024 * 1024),
    )(q.reshape(BH, Sq, D), k.reshape(BH, Sk, D), v.reshape(BH, Sk, D))
    return out.reshape(B, H, Sq, D)
```

```python
import math

import jax
import jax.numpy as jnp
from jax import lax
import jax.experimental.pallas as pl
import jax.experimental.pallas.tpu as pltpu

_NB = 8
_K_ROWS = 128
_V_ROWS = 256


def _kernel(q_hbm, k_hbm, v_hbm, o_hbm,
            qbuf, obuf, kbuf, vbuf, ksem, vsem, qsem, osem):
    bh, _, d = q_hbm.shape
    sk = k_hbm.shape[1]
    c = (d ** -0.5) * math.log2(math.e)
    ratio = _V_ROWS // _K_ROWS

    def start_head(h, slot):
        for j in range(sk // _V_ROWS):
            for i in range(ratio):
                off = (j * ratio + i) * _K_ROWS
                pltpu.make_async_copy(
                    k_hbm.at[h, pl.ds(off, _K_ROWS)],
                    kbuf.at[slot, pl.ds(off, _K_ROWS)],
                    ksem.at[slot]).start(priority=0)
            off = j * _V_ROWS
            pltpu.make_async_copy(
                v_hbm.at[h, pl.ds(off, _V_ROWS)],
                vbuf.at[slot, pl.ds(off, _V_ROWS)],
                vsem.at[slot]).start(priority=1)

    def compute(h, slot):
        pltpu.make_async_copy(kbuf.at[slot], kbuf.at[slot], ksem.at[slot]).wait()
        s = lax.dot_general(qbuf[h], kbuf[slot], (((1,), (1,)), ((), ())),
                            preferred_element_type=jnp.float32)
        m = jnp.max(s, axis=-1, keepdims=True)
        p = jnp.exp2((s - m) * c)
        l = jnp.sum(p, axis=-1, keepdims=True)
        p = p.astype(vbuf.dtype)
        pltpu.make_async_copy(vbuf.at[slot], vbuf.at[slot], vsem.at[slot]).wait()
        o = jnp.dot(p, vbuf[slot], preferred_element_type=jnp.float32)
        obuf[h] = (o / l).astype(obuf.dtype)

    q_copy = pltpu.make_async_copy(q_hbm, qbuf, qsem.at[0])
    q_copy.start()
    for j in range(_NB):
        start_head(j, j)
    q_copy.wait()

    def body(h, carry):
        slot = lax.rem(h, _NB)
        compute(h, slot)

        @pl.when(h + _NB < bh)
        def _():
            start_head(h + _NB, slot)

        return carry

    lax.fori_loop(0, bh - 1, body, 0)

    bulk = pltpu.make_async_copy(
        obuf.at[pl.ds(0, bh - 1)], o_hbm.at[pl.ds(0, bh - 1)], osem.at[0])
    bulk.start()
    compute(bh - 1, (bh - 1) % _NB)
    last = pltpu.make_async_copy(
        obuf.at[pl.ds(bh - 1, 1)], o_hbm.at[pl.ds(bh - 1, 1)], osem.at[1])
    last.start()
    bulk.wait()
    last.wait()


@jax.jit
def pallas_standalone__mha_softmax__sampling_kernel(
    q: jax.Array,
    k: jax.Array,
    v: jax.Array,
):
    B, H, Sq, D = q.shape
    Sk = k.shape[2]
    BH = B * H
    out = pl.pallas_call(
        _kernel,
        in_specs=[pl.BlockSpec(memory_space=pl.ANY)] * 3,
        out_specs=pl.BlockSpec(memory_space=pl.ANY),
        out_shape=jax.ShapeDtypeStruct((BH, Sq, D), q.dtype),
        scratch_shapes=[
            pltpu.VMEM((BH, Sq, D), q.dtype),
            pltpu.VMEM((BH, Sq, D), q.dtype),
            pltpu.VMEM((_NB, Sk, D), k.dtype),
            pltpu.VMEM((_NB, Sk, D), v.dtype),
            pltpu.SemaphoreType.DMA((_NB,)),
            pltpu.SemaphoreType.DMA((_NB,)),
            pltpu.SemaphoreType.DMA((1,)),
            pltpu.SemaphoreType.DMA((2,)),
        ],
        compiler_params=pltpu.CompilerParams(
            vmem_limit_bytes=64 * 1024 * 1024),
    )(q.reshape(BH, Sq, D), k.reshape(BH, Sk, D), v.reshape(BH, Sk, D))
    return out.reshape(B, H, Sq, D)
```

```python
import math

import jax
import jax.numpy as jnp
from jax import lax
import jax.experimental.pallas as pl
import jax.experimental.pallas.tpu as pltpu

_G = 8
_ROWS = 16
_NG = 3
_LAG = 12


def _kernel(q_hbm, k_hbm, v_hbm, o_hbm,
            qbuf, obuf, kbuf, vbuf, ksem, vsem, qsem, osem):
    bh, _, d = q_hbm.shape
    ngrp, _, sk, _ = k_hbm.shape
    c = (d ** -0.5) * math.log2(math.e)
    chunk = sk // _G

    def start_chunk(t):
        g = t // _G
        slot = g % _NG
        base = (t % _G) * chunk
        for i in range(chunk // _ROWS):
            rows = pl.ds(pl.multiple_of(base + i * _ROWS, _ROWS), _ROWS)
            pltpu.make_async_copy(k_hbm.at[g, :, rows], kbuf.at[slot, :, rows],
                                  ksem.at[slot]).start(priority=0)
            pltpu.make_async_copy(v_hbm.at[g, :, rows], vbuf.at[slot, :, rows],
                                  vsem.at[slot]).start(priority=1)

    def wait_group(slot):
        pltpu.make_async_copy(kbuf.at[slot], kbuf.at[slot], ksem.at[slot]).wait()
        pltpu.make_async_copy(vbuf.at[slot], vbuf.at[slot], vsem.at[slot]).wait()

    def compute(h, slot, j):
        s = lax.dot_general(qbuf[h], kbuf[slot, j], (((1,), (1,)), ((), ())),
                            preferred_element_type=jnp.float32)
        m = jnp.max(s, axis=-1, keepdims=True)
        p = jnp.exp2((s - m) * c)
        l = jnp.sum(p, axis=-1, keepdims=True)
        o = jnp.dot(p.astype(vbuf.dtype), vbuf[slot, j],
                    preferred_element_type=jnp.float32)
        obuf[h] = (o / l).astype(obuf.dtype)

    q_copy = pltpu.make_async_copy(q_hbm, qbuf, qsem.at[0])
    q_copy.start()

    def prologue(t, carry):
        start_chunk(t)
        return carry

    lax.fori_loop(0, _LAG, prologue, 0)
    q_copy.wait()

    def body(t, carry):
        j = t % _G
        slot = (t // _G) % _NG

        @pl.when(j == 0)
        def _():
            wait_group(slot)

        compute(t, slot, j)

        @pl.when(t + _LAG < bh)
        def _():
            start_chunk(t + _LAG)

        return carry

    nb = bh - _G
    lax.fori_loop(0, nb, body, 0)

    slot = (ngrp - 1) % _NG
    wait_group(slot)
    bulk = pltpu.make_async_copy(
        obuf.at[pl.ds(0, nb)], o_hbm.at[pl.ds(0, nb)], osem.at[0])
    bulk.start()

    def tail(j, carry):
        compute(nb + j, slot, j)
        return carry

    lax.fori_loop(0, _G, tail, 0)
    last = pltpu.make_async_copy(
        obuf.at[pl.ds(nb, _G)], o_hbm.at[pl.ds(nb, _G)], osem.at[1])
    last.start()
    bulk.wait()
    last.wait()


@jax.jit
def pallas_standalone__mha_softmax__sampling_kernel(
    q: jax.Array,
    k: jax.Array,
    v: jax.Array,
):
    B, H, Sq, D = q.shape
    Sk = k.shape[2]
    BH = B * H
    out = pl.pallas_call(
        _kernel,
        in_specs=[pl.BlockSpec(memory_space=pl.ANY)] * 3,
        out_specs=pl.BlockSpec(memory_space=pl.ANY),
        out_shape=jax.ShapeDtypeStruct((BH, Sq, D), q.dtype),
        scratch_shapes=[
            pltpu.VMEM((BH, Sq, D), q.dtype),
            pltpu.VMEM((BH, Sq, D), q.dtype),
            pltpu.VMEM((_NG, _G, Sk, D), k.dtype),
            pltpu.VMEM((_NG, _G, Sk, D), v.dtype),
            pltpu.SemaphoreType.DMA((_NG,)),
            pltpu.SemaphoreType.DMA((_NG,)),
            pltpu.SemaphoreType.DMA((1,)),
            pltpu.SemaphoreType.DMA((2,)),
        ],
        compiler_params=pltpu.CompilerParams(
            vmem_limit_bytes=64 * 1024 * 1024),
    )(q.reshape(BH, Sq, D),
      k.reshape(BH // _G, _G, Sk, D),
      v.reshape(BH // _G, _G, Sk, D))
    return out.reshape(B, H, Sq, D)
```

```python
import math

import jax
import jax.numpy as jnp
from jax import lax
import jax.experimental.pallas as pl
import jax.experimental.pallas.tpu as pltpu

_G = 8
_ROWS = 16
_NG = 3
_LAG = 12
_KLEAD = 4
_QS = 4
_OH = 4


def _kernel(q_hbm, k_hbm, v_hbm, o_hbm,
            qbuf, obuf, kbuf, vbuf, pbuf, lbuf, ksem, vsem, qsem, osem):
    _, hs, sq, d = q_hbm.shape
    ngrp, _, sk, _ = k_hbm.shape
    bh = ngrp * _G
    c = (d ** -0.5) * math.log2(math.e)
    chunk = sk // _G
    ncopy = chunk // _ROWS

    def kv_copy(src, dst, sems, t, i, sem_idx=None):
        g = t // _G
        slot = g % _NG
        rows = pl.ds(pl.multiple_of((t % _G) * chunk + i * _ROWS, _ROWS), _ROWS)
        return pltpu.make_async_copy(
            src.at[g, :, rows], dst.at[slot, :, rows],
            sems.at[slot if sem_idx is None else sem_idx])

    def start_pairs(t):
        for i in range(ncopy):
            kv_copy(k_hbm, kbuf, ksem, t + _KLEAD, i).start(priority=0)
            kv_copy(v_hbm, vbuf, vsem, t, i).start(priority=1)

    def wait_all(dst, sem):
        pltpu.make_async_copy(dst, dst, sem).wait()

    def scores(h, slot, j):
        s = lax.dot_general(qbuf[h // hs, h % hs], kbuf[slot, j],
                            (((1,), (1,)), ((), ())),
                            preferred_element_type=jnp.float32)
        m = jnp.max(s, axis=-1, keepdims=True)
        p = jnp.exp2((s - m) * c)
        l = jnp.sum(p, axis=-1, keepdims=True)
        return p.astype(vbuf.dtype), l

    def finish(h, slot, j, p, l):
        o = jnp.dot(p, vbuf[slot, j], preferred_element_type=jnp.float32)
        obuf[h // hs, h % hs] = (o / l).astype(obuf.dtype)

    def compute(h, slot, j):
        finish(h, slot, j, *scores(h, slot, j))

    qh = hs // (_KLEAD * ncopy)

    def lead(t, carry):
        for i in range(ncopy):
            kv_copy(k_hbm, kbuf, ksem, t, i).start(priority=0)
            heads = pl.ds((t * ncopy + i) * qh, qh)
            pltpu.make_async_copy(q_hbm.at[:, heads], qbuf.at[:, heads],
                                  qsem.at[0]).start(priority=1)
        return carry

    def fill(t, carry):
        start_pairs(t)
        return carry

    lax.fori_loop(0, _KLEAD, lead, 0)
    lax.fori_loop(0, _LAG, fill, 0)
    wait_all(qbuf, qsem.at[0])

    def body(t, carry):
        j = t % _G
        slot = (t // _G) % _NG

        @pl.when(j == 0)
        def _():
            wait_all(kbuf.at[slot], ksem.at[slot])
            wait_all(vbuf.at[slot], vsem.at[slot])

        compute(t, slot, j)
        start_pairs(t + _LAG)
        return carry

    n_main = bh - _LAG - _KLEAD
    assert n_main == bh - 2 * _G and _G % _KLEAD == 0
    lax.fori_loop(0, n_main, body, 0)

    slot = (ngrp - 2) % _NG
    last_slot = (ngrp - 1) % _NG
    wait_all(kbuf.at[slot], ksem.at[slot])
    wait_all(vbuf.at[slot], vsem.at[slot])
    per = _G // _KLEAD

    def drain(x, carry):
        for u in range(per):
            compute(n_main + x * per + u, slot, x * per + u)
        sem_idx = jnp.where(x == _KLEAD - 1, _NG, last_slot)
        for i in range(ncopy):
            kv_copy(v_hbm, vbuf, vsem, bh - _KLEAD + x, i,
                    sem_idx).start(priority=1)
        return carry

    lax.fori_loop(0, _KLEAD, drain, 0)

    slot = last_slot
    nb = bh - _G
    wait_all(kbuf.at[slot], ksem.at[slot])
    for j in range(_G):
        p, l = scores(nb + j, slot, j)
        pbuf[j] = p
        lbuf[j] = jnp.broadcast_to(l, (sq, d))

    wait_all(vbuf.at[slot, :, pl.ds(0, sk - chunk)], vsem.at[slot])
    writes = []
    for x in range(0, hs, _OH):
        segs = pl.ds(0, _QS if x < hs - _G else _QS - 1)
        writes.append(pltpu.make_async_copy(
            obuf.at[segs, pl.ds(x, _OH)], o_hbm.at[segs, pl.ds(x, _OH)],
            osem.at[0]))
        writes[-1].start()
    wait_all(vbuf.at[slot, :, pl.ds(sk - chunk, chunk)], vsem.at[_NG])
    for j in range(_G):
        finish(nb + j, slot, j, pbuf[j], lbuf[j])
    writes.append(pltpu.make_async_copy(
        obuf.at[_QS - 1, pl.ds(hs - _G, _G)],
        o_hbm.at[_QS - 1, pl.ds(hs - _G, _G)], osem.at[1]))
    writes[-1].start()
    for w in writes:
        w.wait()


@jax.jit
def pallas_standalone__mha_softmax__sampling_kernel(
    q: jax.Array,
    k: jax.Array,
    v: jax.Array,
):
    B, H, Sq, D = q.shape
    Sk = k.shape[2]
    BH = B * H
    q_shape = (_QS, BH // _QS, Sq, D)
    kv_shape = (BH // _G, _G, Sk, D)
    out = pl.pallas_call(
        _kernel,
        in_specs=[pl.BlockSpec(memory_space=pl.ANY)] * 3,
        out_specs=pl.BlockSpec(memory_space=pl.ANY),
        out_shape=jax.ShapeDtypeStruct(q_shape, q.dtype),
        scratch_shapes=[
            pltpu.VMEM(q_shape, q.dtype),
            pltpu.VMEM(q_shape, q.dtype),
            pltpu.VMEM((_NG, _G, Sk, D), k.dtype),
            pltpu.VMEM((_NG, _G, Sk, D), v.dtype),
            pltpu.VMEM((_G, Sq, Sk), v.dtype),
            pltpu.VMEM((_G, Sq, D), jnp.float32),
            pltpu.SemaphoreType.DMA((_NG,)),
            pltpu.SemaphoreType.DMA((_NG + 1,)),
            pltpu.SemaphoreType.DMA((1,)),
            pltpu.SemaphoreType.DMA((2,)),
        ],
        compiler_params=pltpu.CompilerParams(
            vmem_limit_bytes=64 * 1024 * 1024),
    )(q.reshape(q_shape), k.reshape(kv_shape), v.reshape(kv_shape))
    return out.reshape(B, H, Sq, D)
```
